```python
import jax
import jax.numpy as jnp

def _softmax(x, axis=-1):
    return jax.nn.softmax(x, axis=axis)

def _gelu(x):
    return jax.nn.gelu(x, approximate=True)

def _silu(x):
    return jax.nn.silu(x)

def _sigmoid(x):
    return jax.nn.sigmoid(x)

def _layernorm(x, axis=-1, eps=1e-05):
    m = jnp.mean(x, axis=axis, keepdims=True)
    v = jnp.var(x, axis=axis, keepdims=True)
    return (x - m) / jnp.sqrt(v + eps)

def _scatter_add(tgt, idx, src, axis=0):
    return tgt.at[idx].add(src)

def _segment_sum(src, seg, n):
    return jax.ops.segment_sum(src, seg, n)

class _Rng:

    def __init__(self, key):
        self._k = key

    def _next(self):
        self._k, sub = jax.random.split(self._k)
        return sub

    def normal(self, shape):
        return jax.random.normal(self._next(), shape, dtype=jnp.bfloat16)

    def randint(self, lo, hi, shape):
        return jax.random.randint(self._next(), shape, lo, hi, dtype=jnp.int32)

    def uniform(self, shape, lo=0.0, hi=1.0):
        return jax.random.uniform(self._next(), shape, jnp.bfloat16, lo, hi)

    def permutation(self, n):
        return jax.random.permutation(self._next(), n)
kernel_name = 'adaLN_cond__sliding_block_cached__mixer_gmlp__decode'

def setup_inputs():
    _rng = _Rng(jax.random.key(int.from_bytes(__import__("os").urandom(4), "little")))
    _w = lambda a: (lambda t: t.astype(jnp.bfloat16) if jnp.issubdtype(t.dtype, jnp.floating) else t)(jnp.asarray(a))

    def _A_setup():
        B, Sq, D = (1, 1, 448)
        Hq, Hkv, Sk, Dh = (16, 8, 65536, 256)
        assert Hq % Hkv == 0, (Hq, Hkv)
        return {'x': _w((lambda *s: _rng.normal(s) * 0.05)(B, Sq, D)), 'k_cache': _w((lambda *s: _rng.normal(s) * 0.05)(B, Hkv, Sk, Dh)), 'v_cache': _w((lambda *s: _rng.normal(s) * 0.05)(B, Hkv, Sk, Dh)), 'wq': _w((lambda *s: _rng.normal(s) * 0.05)(D, Hq * Dh) * D ** (-0.5)), 'wo': _w((lambda *s: _rng.normal(s) * 0.05)(Hq * Dh, D) * (Hq * Dh) ** (-0.5))}
    _A_in = _A_setup()

    def _B_setup():
        B, S, D, F = (1, 1, 448, 1792)
        Fh = F // 2
        return {'x': _w((lambda *s: _rng.normal(s) * 0.05)(B, S, D)), 'w_in': _w((lambda *s: _rng.normal(s) * 0.05)(D, 2 * Fh)), 'w_sp': _w(0.01 * (lambda *s: _rng.normal(s) * 0.05)(S, S)), 'b_sp': _w(1.0 + 0.01 * (lambda *s: _rng.normal(s) * 0.05)(S)), 'w_out': _w((lambda *s: _rng.normal(s) * 0.05)(Fh, D))}
    _B_in = _B_setup()
    return {'A_x': _A_in['x'], 'A_k_cache': _A_in['k_cache'], 'A_v_cache': _A_in['v_cache'], 'A_wq': _A_in['wq'], 'A_wo': _A_in['wo'], 'B_x': _B_in['x'], 'B_w_in': _B_in['w_in'], 'B_w_sp': _B_in['w_sp'], 'B_b_sp': _B_in['b_sp'], 'B_w_out': _B_in['w_out'], 'c': _w((lambda *s: _rng.normal(s) * 0.05)(1, 448)), 'w_mod': _w((lambda *s: _rng.normal(s) * 0.05)(448, 6 * 448) * 448 ** (-0.5))}

def reference(A_x, A_k_cache, A_v_cache, A_wq, A_wo, B_x, B_w_in, B_w_sp, B_b_sp, B_w_out, c, w_mod):

    def _A_ref(x, k_cache, v_cache, wq, wo):
        B, Sq, D = x.shape
        Hq, Dh = (16, 256)
        Hkv, Sk = (k_cache.shape[1], k_cache.shape[2])
        W = min(4096, max(256, Sk // 4))
        rep = Hq // Hkv
        q = (lambda x, *d: x.transpose(*d))((x @ wq).reshape(B, Sq, Hq, Dh), 0, 2, 1, 3)
        k = jnp.repeat(k_cache[:, :, Sk - W:, :], rep, axis=1)
        v = jnp.repeat(v_cache[:, :, Sk - W:, :], rep, axis=1)
        scores = jnp.einsum('bhqd,bhkd->bhqk', q, k) * Dh ** (-0.5)
        p = _softmax(scores, axis=-1)
        o = jnp.einsum('bhqk,bhkd->bhqd', p, v)
        return (lambda x, *d: x.transpose(*d))(o, 0, 2, 1, 3).reshape(B, Sq, Hq * Dh) @ wo

    def _B_ref(x, w_in, w_sp, b_sp, w_out):
        B, S, D = x.shape
        F = w_in.shape[-1]
        Fh = F // 2
        z = _gelu(jnp.einsum('bsd,df->bsf', x, w_in))
        z1 = z[..., :Fh].copy()
        z2 = _layernorm(z[..., Fh:], axis=-1)
        g = jnp.einsum('ts,bsf->btf', w_sp, z2) + b_sp[None, :, None]
        return jnp.einsum('bsf,fd->bsd', z1 * g, w_out)
    x = A_x
    mod = (_silu(c) @ w_mod).reshape(c.shape[0], 6, 1, -1)
    sa, ca, ga, sb, cb, gb = (mod[:, 0].copy(), mod[:, 1].copy(), mod[:, 2].copy(), mod[:, 3].copy(), mod[:, 4].copy(), mod[:, 5].copy())
    h = _layernorm(x, axis=-1) * (1 + ca) + sa
    x = x + ga * _A_ref(h, A_k_cache, A_v_cache, A_wq, A_wo)
    h = _layernorm(x, axis=-1) * (1 + cb) + sb
    x = x + gb * _B_ref(h, B_w_in, B_w_sp, B_b_sp, B_w_out)
    return x
```

```python
import jax
import jax.numpy as jnp
from jax import lax
import jax.experimental.pallas as pl
import jax.experimental.pallas.tpu as pltpu

_HQ, _DH = 16, 256
_EPS = 1e-5
_M = 8

_NT = (((1,), (1,)), ((), ()))


def _layernorm(x):
    mean = jnp.mean(x, axis=-1, keepdims=True)
    d = x - mean
    var = jnp.mean(d * d, axis=-1, keepdims=True)
    return d * lax.rsqrt(var + _EPS)


def _gelu_tanh(x):
    inner = 0.7978845608028654 * (x + 0.044715 * (x * x * x))
    return 0.5 * x * (1.0 + jnp.tanh(inner))


def _rows(v):
    return jnp.broadcast_to(v, (_M, v.shape[-1]))


@jax.jit
def pallas_adaLN_cond__sliding_block_cached__mixer_gmlp__decode_kernel(
    A_x: jax.Array,
    A_k_cache: jax.Array,
    A_v_cache: jax.Array,
    A_wq: jax.Array,
    A_wo: jax.Array,
    B_x: jax.Array,
    B_w_in: jax.Array,
    B_w_sp: jax.Array,
    B_b_sp: jax.Array,
    B_w_out: jax.Array,
    c: jax.Array,
    w_mod: jax.Array,
):
    del B_x
    D = A_x.shape[-1]
    HKV, SK = A_k_cache.shape[1], A_k_cache.shape[2]
    W = min(4096, max(256, SK // 4))
    REP = _HQ // HKV
    assert REP == 2
    F = B_w_in.shape[-1]
    FH = F // 2
    bf16, f32 = jnp.bfloat16, jnp.float32

    def kernel(x_hbm, k_hbm, v_hbm, wq_hbm, woT_hbm, win_hbm, wsp_hbm, bsp_hbm,
               woutT_hbm, c_hbm, wmod_hbm,
               out_ref,
               x_v, c_v, wsp_v, bsp_v, wmod_v, wq_v, k_v, v_v, woT_v, win_v,
               woutT_v, q_s, o_s, sem_w, sem_k, sem_v):
        def k_copy(g):
            return pltpu.make_async_copy(
                k_hbm.at[0, g, pl.ds(SK - W, W), :], k_v.at[g], sem_k.at[g])

        def v_copy(g):
            return pltpu.make_async_copy(
                v_hbm.at[0, g, pl.ds(SK - W, W), :], v_v.at[g], sem_v.at[g])

        wmod_cp = pltpu.make_async_copy(wmod_hbm, wmod_v, sem_w.at[0])
        c_cp = pltpu.make_async_copy(c_hbm, c_v, sem_w.at[1])
        x_cp = pltpu.make_async_copy(x_hbm.at[0], x_v, sem_w.at[2])
        wq_cp = pltpu.make_async_copy(wq_hbm, wq_v, sem_w.at[3])
        wo_cp = pltpu.make_async_copy(woT_hbm, woT_v, sem_w.at[4])
        win_cp = pltpu.make_async_copy(win_hbm, win_v, sem_w.at[5])
        wsp_cp = pltpu.make_async_copy(wsp_hbm, wsp_v, sem_w.at[6])
        bsp_cp = pltpu.make_async_copy(bsp_hbm, bsp_v, sem_w.at[7])
        wout_cp = pltpu.make_async_copy(woutT_hbm, woutT_v, sem_w.at[8])

        wmod_cp.start()
        c_cp.start()
        x_cp.start()
        wq_cp.start()
        for g in range(HKV):
            k_copy(g).start()
            v_copy(g).start()
        wo_cp.start()
        wsp_cp.start()
        bsp_cp.start()
        win_cp.start()
        wout_cp.start()

        c_cp.wait()
        cf = c_v[...].astype(f32)
        sc = _rows(cf * jax.nn.sigmoid(cf)).astype(bf16)
        wmod_cp.wait()
        mod = jnp.dot(sc, wmod_v[...], preferred_element_type=f32)
        sa, ca, ga, sb, cb, gb = (mod[:, i * D:(i + 1) * D] for i in range(6))

        x_cp.wait()
        x0 = _rows(x_v[...].astype(f32))
        h = (_layernorm(x0) * (1.0 + ca) + sa).astype(bf16)
        wq_cp.wait()
        q = jnp.dot(h, wq_v[...], preferred_element_type=f32)
        even = (lax.broadcasted_iota(jnp.int32, (_M, _DH), 0) % 2) == 0
        for g in range(HKV):
            qa = q[:, (2 * g) * _DH:(2 * g + 1) * _DH]
            qb = q[:, (2 * g + 1) * _DH:(2 * g + 2) * _DH]
            q_s[g] = jnp.where(even, qa, qb).astype(bf16)

        def head(g, carry):
            k_copy(g).wait()
            s = lax.dot_general(q_s[g], k_v[g], _NT,
                                preferred_element_type=f32) * (_DH ** -0.5)
            m = jnp.max(s, axis=-1, keepdims=True)
            p = jnp.exp(s - m)
            l = jnp.sum(p, axis=-1, keepdims=True)
            v_copy(g).wait()
            o = jnp.dot(p.astype(bf16), v_v[g], preferred_element_type=f32)
            o_s[g] = o / l
            return carry

        lax.fori_loop(0, HKV, head, 0)

        parts = []
        for g in range(HKV):
            o = o_s[g]
            parts.append(jnp.where(even, o, 0.0))
            parts.append(jnp.where(even, 0.0, o))
        o_all = jnp.concatenate(parts, axis=-1).astype(bf16)
        wo_cp.wait()
        y = lax.dot_general(o_all, woT_v[...], _NT, preferred_element_type=f32)
        y = _rows(y[0:1] + y[1:2])
        x1 = x0 + ga * y

        h2 = (_layernorm(x1) * (1.0 + cb) + sb).astype(bf16)
        win_cp.wait()
        z = _gelu_tanh(jnp.dot(h2, win_v[...], preferred_element_type=f32))
        z1, z2 = z[:, :FH], _layernorm(z[:, FH:])
        wsp_cp.wait()
        bsp_cp.wait()
        gate = wsp_v[...].astype(f32) * z2 + bsp_v[...].astype(f32)
        zg = (z1 * gate).astype(bf16)
        wout_cp.wait()
        y2 = lax.dot_general(zg, woutT_v[...], _NT, preferred_element_type=f32)
        x2 = x1 + gb * y2
        out_ref[0] = x2[0:1].astype(out_ref.dtype)

    any_spec = pl.BlockSpec(memory_space=pl.ANY)
    return pl.pallas_call(
        kernel,
        out_shape=jax.ShapeDtypeStruct(A_x.shape, A_x.dtype),
        in_specs=[any_spec] * 11,
        out_specs=pl.BlockSpec(memory_space=pltpu.VMEM),
        scratch_shapes=[
            pltpu.VMEM((1, D), bf16),
            pltpu.VMEM((1, D), bf16),
            pltpu.VMEM((1, 1), bf16),
            pltpu.VMEM((1, 1), bf16),
            pltpu.VMEM((D, 6 * D), bf16),
            pltpu.VMEM((D, _HQ * _DH), bf16),
            pltpu.VMEM((HKV, W, _DH), bf16),
            pltpu.VMEM((HKV, W, _DH), bf16),
            pltpu.VMEM((D, _HQ * _DH), bf16),
            pltpu.VMEM((D, F), bf16),
            pltpu.VMEM((D, FH), bf16),
            pltpu.VMEM((HKV, _M, _DH), bf16),
            pltpu.VMEM((HKV, _M, _DH), f32),
            pltpu.SemaphoreType.DMA((9,)),
            pltpu.SemaphoreType.DMA((HKV,)),
            pltpu.SemaphoreType.DMA((HKV,)),
        ],
        compiler_params=pltpu.CompilerParams(
            vmem_limit_bytes=100 * 1024 * 1024),
    )(A_x, A_k_cache, A_v_cache, A_wq, A_wo.T, B_w_in, B_w_sp,
      B_b_sp.reshape(1, 1), B_w_out.T, c, w_mod)
```

```python
import jax
import jax.numpy as jnp
from jax import lax
import jax.experimental.pallas as pl
import jax.experimental.pallas.tpu as pltpu

_HQ, _DH = 16, 256
_EPS = 1e-5
_M = 8
_ROWS = 128

_NT = (((1,), (1,)), ((), ()))


def _layernorm(x):
    mean = jnp.mean(x, axis=-1, keepdims=True)
    d = x - mean
    var = jnp.mean(d * d, axis=-1, keepdims=True)
    return d * lax.rsqrt(var + _EPS)


def _gelu_tanh(x):
    inner = 0.7978845608028654 * (x + 0.044715 * (x * x * x))
    return 0.5 * x * (1.0 + jnp.tanh(inner))


def _rows(v):
    return jnp.broadcast_to(v, (_M, v.shape[-1]))


@jax.jit
def pallas_adaLN_cond__sliding_block_cached__mixer_gmlp__decode_kernel(
    A_x: jax.Array,
    A_k_cache: jax.Array,
    A_v_cache: jax.Array,
    A_wq: jax.Array,
    A_wo: jax.Array,
    B_x: jax.Array,
    B_w_in: jax.Array,
    B_w_sp: jax.Array,
    B_b_sp: jax.Array,
    B_w_out: jax.Array,
    c: jax.Array,
    w_mod: jax.Array,
):
    del B_x
    D = A_x.shape[-1]
    HKV, SK = A_k_cache.shape[1], A_k_cache.shape[2]
    W = min(4096, max(256, SK // 4))
    assert A_x.shape == (1, 1, 448) and _HQ == 2 * HKV
    F = B_w_in.shape[-1]
    FH = F // 2
    bf16, f32 = jnp.bfloat16, jnp.float32
    out_chunks = ((0, 2 * _ROWS), (2 * _ROWS, _ROWS), (3 * _ROWS, D - 3 * _ROWS))

    def kernel(x_hbm, k_hbm, v_hbm, wq_hbm, woT_hbm, win_hbm, wsp_hbm, bsp_hbm,
               woutT_hbm, c_hbm, wmod_hbm,
               out_ref,
               x_v, c_v, wsp_v, bsp_v, wmod_v, wq_v, k_v, v_v, woT_v, win_v,
               woutT_v, q_s, o_s, mod_s):

        def body(sem_w, sem_kv, sem_out):
            def k_copy(g):
                return pltpu.make_async_copy(
                    k_hbm.at[0, g, pl.ds(SK - W, W), :], k_v.at[g], sem_kv.at[g])

            def v_copy(g):
                return pltpu.make_async_copy(
                    v_hbm.at[0, g, pl.ds(SK - W, W), :], v_v.at[g], sem_kv.at[g])

            def wout_copy(i):
                r0, n = out_chunks[i]
                return pltpu.make_async_copy(
                    woutT_hbm.at[pl.ds(r0, n), :], woutT_v.at[pl.ds(r0, n), :],
                    sem_out.at[i])

            first = [
                pltpu.make_async_copy(wmod_hbm, wmod_v, sem_w.at[0]),
                pltpu.make_async_copy(c_hbm, c_v, sem_w.at[0]),
                pltpu.make_async_copy(x_hbm.at[0], x_v, sem_w.at[0]),
                pltpu.make_async_copy(wq_hbm, wq_v, sem_w.at[0]),
                pltpu.make_async_copy(wsp_hbm, wsp_v, sem_w.at[0]),
                pltpu.make_async_copy(bsp_hbm, bsp_v, sem_w.at[0]),
            ]
            wo_cp = pltpu.make_async_copy(woT_hbm, woT_v, sem_w.at[1])
            win_cp = pltpu.make_async_copy(win_hbm, win_v, sem_w.at[2])
            late = [wo_cp, win_cp] + [wout_copy(i) for i in range(len(out_chunks))]
            assert len(late) <= HKV

            for cp in first:
                cp.start()

            def issue_kv(g, carry):
                k_copy(g).start()
                v_copy(g).start()
                return carry

            lax.fori_loop(0, HKV, issue_kv, 0)

            for cp in first:
                cp.wait()
            cf = c_v[...].astype(f32)
            sc = _rows(cf * jax.nn.sigmoid(cf)).astype(bf16)
            mod = jnp.dot(sc, wmod_v[...], preferred_element_type=f32)
            for i in range(6):
                mod_s[i] = mod[:, i * D:(i + 1) * D]

            x0 = _rows(x_v[...].astype(f32))
            h = (_layernorm(x0) * (1.0 + mod_s[1]) + mod_s[0]).astype(bf16)
            q = jnp.dot(h, wq_v[...], preferred_element_type=f32)
            even = (lax.broadcasted_iota(jnp.int32, (_M, _DH), 0) % 2) == 0
            for g in range(HKV):
                qa = q[:, (2 * g) * _DH:(2 * g + 1) * _DH]
                qb = q[:, (2 * g + 1) * _DH:(2 * g + 2) * _DH]
                q_s[g] = jnp.where(even, qa, qb).astype(bf16)

            def head(g, carry):
                k_copy(g).wait()
                v_copy(g).wait()
                for i, cp in enumerate(late):
                    pl.when(g == i)(cp.start)
                s = lax.dot_general(q_s[g], k_v[g], _NT,
                                    preferred_element_type=f32) * (_DH ** -0.5)
                m = jnp.max(s, axis=-1, keepdims=True)
                p = jnp.exp(s - m)
                l = jnp.sum(p, axis=-1, keepdims=True)
                o = jnp.dot(p.astype(bf16), v_v[g], preferred_element_type=f32)
                o_s[g] = o / l
                return carry

            lax.fori_loop(0, HKV, head, 0)

            parts = []
            for g in range(HKV):
                o = o_s[g]
                parts.append(jnp.where(even, o, 0.0))
                parts.append(jnp.where(even, 0.0, o))
            o_all = jnp.concatenate(parts, axis=-1).astype(bf16)
            wo_cp.wait()
            y = lax.dot_general(o_all, woT_v[...], _NT, preferred_element_type=f32)
            y = _rows(y[0:1] + y[1:2])
            x1 = x0 + mod_s[2] * y

            h2 = (_layernorm(x1) * (1.0 + mod_s[4]) + mod_s[3]).astype(bf16)
            win_cp.wait()
            z = _gelu_tanh(jnp.dot(h2, win_v[...], preferred_element_type=f32))
            z1, z2 = z[:, :FH], _layernorm(z[:, FH:])
            gate = wsp_v[...].astype(f32) * z2 + bsp_v[...].astype(f32)
            zg = (z1 * gate).astype(bf16)
            y2 = []
            for i, (r0, n) in enumerate(out_chunks):
                wout_copy(i).wait()
                y2.append(lax.dot_general(zg, woutT_v[r0:r0 + n, :], _NT,
                                          preferred_element_type=f32))
            x2 = x1 + mod_s[5] * jnp.concatenate(y2, axis=-1)
            out_ref[0] = x2[0:1].astype(out_ref.dtype)

        pl.run_scoped(
            body,
            pltpu.SemaphoreType.DMA((3,)),
            pltpu.SemaphoreType.DMA((HKV,)),
            pltpu.SemaphoreType.DMA((len(out_chunks),)),
        )

    any_spec = pl.BlockSpec(memory_space=pl.ANY)
    return pl.pallas_call(
        kernel,
        out_shape=jax.ShapeDtypeStruct(A_x.shape, A_x.dtype),
        in_specs=[any_spec] * 11,
        out_specs=pl.BlockSpec(memory_space=pltpu.VMEM),
        scratch_shapes=[
            pltpu.VMEM((1, D), bf16),
            pltpu.VMEM((1, D), bf16),
            pltpu.VMEM((1, 1), bf16),
            pltpu.VMEM((1, 1), bf16),
            pltpu.VMEM((D, 6 * D), bf16),
            pltpu.VMEM((D, _HQ * _DH), bf16),
            pltpu.VMEM((HKV, W, _DH), bf16),
            pltpu.VMEM((HKV, W, _DH), bf16),
            pltpu.VMEM((D, _HQ * _DH), bf16),
            pltpu.VMEM((D, F), bf16),
            pltpu.VMEM((D, FH), bf16),
            pltpu.VMEM((HKV, _M, _DH), bf16),
            pltpu.VMEM((HKV, _M, _DH), f32),
            pltpu.VMEM((6, _M, D), f32),
        ],
        compiler_params=pltpu.CompilerParams(
            vmem_limit_bytes=100 * 1024 * 1024),
    )(A_x, A_k_cache, A_v_cache, A_wq, A_wo.T, B_w_in, B_w_sp,
      B_b_sp.reshape(1, 1), B_w_out.T, c, w_mod)
```

```python
import jax
import jax.numpy as jnp
from jax import lax
import jax.experimental.pallas as pl
import jax.experimental.pallas.tpu as pltpu

_HQ, _DH = 16, 256
_EPS = 1e-5
_M = 8
_KV_ROWS = 96

_NT = (((1,), (1,)), ((), ()))


def _layernorm(x):
    mean = jnp.mean(x, axis=-1, keepdims=True)
    d = x - mean
    var = jnp.mean(d * d, axis=-1, keepdims=True)
    return d * lax.rsqrt(var + _EPS)


def _gelu_tanh(x):
    inner = 0.7978845608028654 * (x + 0.044715 * (x * x * x))
    return 0.5 * x * (1.0 + jnp.tanh(inner))


def _rows(v):
    return jnp.broadcast_to(v, (_M, v.shape[-1]))


@jax.jit
def pallas_adaLN_cond__sliding_block_cached__mixer_gmlp__decode_kernel(
    A_x: jax.Array,
    A_k_cache: jax.Array,
    A_v_cache: jax.Array,
    A_wq: jax.Array,
    A_wo: jax.Array,
    B_x: jax.Array,
    B_w_in: jax.Array,
    B_w_sp: jax.Array,
    B_b_sp: jax.Array,
    B_w_out: jax.Array,
    c: jax.Array,
    w_mod: jax.Array,
):
    del B_x
    D = A_x.shape[-1]
    HKV, SK = A_k_cache.shape[1], A_k_cache.shape[2]
    W = min(4096, max(256, SK // 4))
    QD = _HQ * _DH
    F = B_w_in.shape[-1]
    FH = F // 2
    assert A_x.shape == (1, 1, 448) and _HQ == 2 * HKV and F == 1792 and W == 4096
    bf16, f32 = jnp.bfloat16, jnp.float32

    n_full, rem = divmod(W, _KV_ROWS)
    n_kv = n_full + (1 if rem else 0)
    wo_a_rows = 192
    win_a_rows = 224
    out_chunks = ((0, 256), (256, 128), (384, D - 384))

    def kernel(x_hbm, k_hbm, v_hbm, wq_hbm, woT_hbm, win_hbm, wsp_hbm, bsp_hbm,
               woutT_hbm, c_hbm, wmod_hbm,
               out_ref,
               x_v, c_v, wsp_v, bsp_v, wmod_v, wq_v, k_v, v_v, woT_v, win_v,
               woutT_v, q_s, o_s, mod_s):

        def body(sem_w, sem_k, sem_v, sem_out, sem_small):
            def pieces(src, dst, sem, r_lo, r_hi, r_step, c_step):
                return [(src.at[pl.ds(r, r_step), pl.ds(c0, c_step)],
                         dst.at[pl.ds(r, r_step), pl.ds(c0, c_step)], sem)
                        for r in range(r_lo, r_hi, r_step)
                        for c0 in range(0, src.shape[1], c_step)]

            def kv_piece(src, dst, sem, g, r, n):
                return (src.at[0, g, pl.ds(SK - W + r, n), :],
                        dst.at[g, pl.ds(r, n), :], sem.at[g])

            def kv_pieces(src, dst, sem, g):
                out = [kv_piece(src, dst, sem, g, j * _KV_ROWS, _KV_ROWS)
                       for j in range(n_full)]
                if rem:
                    out.append(kv_piece(src, dst, sem, g, W - rem, rem))
                return out

            def start(piece, priority):
                pltpu.make_async_copy(*piece).start(priority=priority)

            def start_pairs(a, b):
                for i in range(max(len(a), len(b))):
                    if i < len(a):
                        start(a[i], 0)
                    if i < len(b):
                        start(b[i], 1)

            def start_kv_pairs(gk, gv):
                def pair(j, carry):
                    r = pl.multiple_of(j * _KV_ROWS, 8)
                    start(kv_piece(k_hbm, k_v, sem_k, gk, r, _KV_ROWS), 0)
                    start(kv_piece(v_hbm, v_v, sem_v, gv, r, _KV_ROWS), 1)
                    return carry

                lax.fori_loop(0, n_full, pair, 0)
                if rem:
                    start(kv_piece(k_hbm, k_v, sem_k, gk, W - rem, rem), 0)
                    start(kv_piece(v_hbm, v_v, sem_v, gv, W - rem, rem), 1)

            def wait_filled(dst, sem):
                pltpu.make_async_copy(dst, dst, sem).wait()

            wmod_p = pieces(wmod_hbm, wmod_v, sem_w.at[0], 0, D, 8, 6 * D)
            wq_p = pieces(wq_hbm, wq_v, sem_w.at[1], 0, D, 8, QD // 2)
            wo_a = pieces(woT_hbm, woT_v, sem_w.at[2], 0, wo_a_rows, 8, QD // 2)
            wo_b = pieces(woT_hbm, woT_v, sem_w.at[2], wo_a_rows, D, 8, QD // 2)
            win_a = pieces(win_hbm, win_v, sem_w.at[3], 0, win_a_rows, 8, F)
            win_b = pieces(win_hbm, win_v, sem_w.at[3], win_a_rows, D, 8, F)
            wout_p = []
            for i, (r0, n) in enumerate(out_chunks):
                wout_p += pieces(woutT_hbm, woutT_v, sem_out.at[i], r0, r0 + n, 16, FH)
            late_a = wo_a + win_a
            late_b = wo_b + win_b + wout_p
            small = [
                pltpu.make_async_copy(c_hbm, c_v, sem_small.at[0]),
                pltpu.make_async_copy(x_hbm.at[0], x_v, sem_small.at[1]),
                pltpu.make_async_copy(wsp_hbm, wsp_v, sem_small.at[2]),
                pltpu.make_async_copy(bsp_hbm, bsp_v, sem_small.at[3]),
            ]

            nb = (len(wq_p) - len(wmod_p) - (n_kv - 1)) // 2
            first_a = wq_p[:len(wq_p) - nb]
            first_b = wmod_p + wq_p[len(wq_p) - nb:]
            start_pairs(first_a[:len(first_b)], first_b)
            start_pairs(first_a[len(first_b):], kv_pieces(v_hbm, v_v, sem_v, 0))
            for cp in small:
                cp.start()
            start_pairs(kv_pieces(k_hbm, k_v, sem_k, 0),
                        kv_pieces(v_hbm, v_v, sem_v, 1))

            for cp in small:
                cp.wait()
            wait_filled(wmod_v, sem_w.at[0])
            wait_filled(wq_v, sem_w.at[1])
            cf = c_v[...].astype(f32)
            sc = _rows(cf * jax.nn.sigmoid(cf)).astype(bf16)
            mod = jnp.dot(sc, wmod_v[...], preferred_element_type=f32)
            for i in range(6):
                mod_s[i] = mod[:, i * D:(i + 1) * D]

            x0 = _rows(x_v[...].astype(f32))
            h = (_layernorm(x0) * (1.0 + mod_s[1]) + mod_s[0]).astype(bf16)
            q = jnp.dot(h, wq_v[...], preferred_element_type=f32)
            even = (lax.broadcasted_iota(jnp.int32, (_M, _DH), 0) % 2) == 0
            for g in range(HKV):
                qa = q[:, (2 * g) * _DH:(2 * g + 1) * _DH]
                qb = q[:, (2 * g + 1) * _DH:(2 * g + 2) * _DH]
                q_s[g] = jnp.where(even, qa, qb).astype(bf16)

            n_a1 = len(wo_a)

            def head(g, carry):
                @pl.when(g + 2 < HKV)
                def _():
                    start_kv_pairs(g + 1, g + 2)

                @pl.when(g + 2 == HKV)
                def _():
                    start_pairs(kv_pieces(k_hbm, k_v, sem_k, HKV - 1), late_b[:n_kv])

                @pl.when(g + 1 == HKV)
                def _():
                    start_pairs(late_a[:n_a1], late_b[n_kv:n_kv + n_a1])

                wait_filled(k_v.at[g], sem_k.at[g])
                wait_filled(v_v.at[g], sem_v.at[g])
                s = lax.dot_general(q_s[g], k_v[g], _NT,
                                    preferred_element_type=f32) * (_DH ** -0.5)
                m = jnp.max(s, axis=-1, keepdims=True)
                p = jnp.exp(s - m)
                l = jnp.sum(p, axis=-1, keepdims=True)
                o = jnp.dot(p.astype(bf16), v_v[g], preferred_element_type=f32)
                o_s[g] = o / l
                return carry

            lax.fori_loop(0, HKV, head, 0)
            start_pairs(late_a[n_a1:], late_b[n_kv + n_a1:])

            parts = []
            for g in range(HKV):
                o = o_s[g]
                parts.append(jnp.where(even, o, 0.0))
                parts.append(jnp.where(even, 0.0, o))
            o_all = jnp.concatenate(parts, axis=-1).astype(bf16)
            wait_filled(woT_v, sem_w.at[2])
            y = lax.dot_general(o_all, woT_v[...], _NT, preferred_element_type=f32)
            y = _rows(y[0:1] + y[1:2])
            x1 = x0 + mod_s[2] * y

            h2 = (_layernorm(x1) * (1.0 + mod_s[4]) + mod_s[3]).astype(bf16)
            wait_filled(win_v, sem_w.at[3])
            z = _gelu_tanh(jnp.dot(h2, win_v[...], preferred_element_type=f32))
            z1, z2 = z[:, :FH], _layernorm(z[:, FH:])
            gate = wsp_v[...].astype(f32) * z2 + bsp_v[...].astype(f32)
            zg = (z1 * gate).astype(bf16)
            y2 = []
            for i, (r0, n) in enumerate(out_chunks):
                wait_filled(woutT_v.at[pl.ds(r0, n), :], sem_out.at[i])
                y2.append(lax.dot_general(zg, woutT_v[r0:r0 + n, :], _NT,
                                          preferred_element_type=f32))
            x2 = x1 + mod_s[5] * jnp.concatenate(y2, axis=-1)
            out_ref[0] = x2[0:1].astype(out_ref.dtype)

        pl.run_scoped(
            body,
            pltpu.SemaphoreType.DMA((4,)),
            pltpu.SemaphoreType.DMA((HKV,)),
            pltpu.SemaphoreType.DMA((HKV,)),
            pltpu.SemaphoreType.DMA((len(out_chunks),)),
            pltpu.SemaphoreType.DMA((4,)),
        )

    any_spec = pl.BlockSpec(memory_space=pl.ANY)
    return pl.pallas_call(
        kernel,
        out_shape=jax.ShapeDtypeStruct(A_x.shape, A_x.dtype),
        in_specs=[any_spec] * 11,
        out_specs=pl.BlockSpec(memory_space=pltpu.VMEM),
        scratch_shapes=[
            pltpu.VMEM((1, D), bf16),
            pltpu.VMEM((1, D), bf16),
            pltpu.VMEM((1, 1), bf16),
            pltpu.VMEM((1, 1), bf16),
            pltpu.VMEM((D, 6 * D), bf16),
            pltpu.VMEM((D, QD), bf16),
            pltpu.VMEM((HKV, W, _DH), bf16),
            pltpu.VMEM((HKV, W, _DH), bf16),
            pltpu.VMEM((D, QD), bf16),
            pltpu.VMEM((D, F), bf16),
            pltpu.VMEM((D, FH), bf16),
            pltpu.VMEM((HKV, _M, _DH), bf16),
            pltpu.VMEM((HKV, _M, _DH), f32),
            pltpu.VMEM((6, _M, D), f32),
        ],
        compiler_params=pltpu.CompilerParams(
            vmem_limit_bytes=100 * 1024 * 1024),
    )(A_x, A_k_cache, A_v_cache, A_wq, A_wo.T, B_w_in, B_w_sp,
      B_b_sp.reshape(1, 1), B_w_out.T, c, w_mod)
```

```python
import jax
import jax.numpy as jnp
from jax import lax
import jax.experimental.pallas as pl
import jax.experimental.pallas.tpu as pltpu

_HQ, _DH = 16, 256
_EPS = 1e-5
_M = 8
_KV_ROWS = 96

_NT = (((1,), (1,)), ((), ()))


def _layernorm(x):
    mean = jnp.mean(x, axis=-1, keepdims=True)
    d = x - mean
    var = jnp.mean(d * d, axis=-1, keepdims=True)
    return d * lax.rsqrt(var + _EPS)


def _gelu_tanh(x):
    inner = 0.7978845608028654 * (x + 0.044715 * (x * x * x))
    return 0.5 * x * (1.0 + jnp.tanh(inner))


def _rows(v):
    return jnp.broadcast_to(v, (_M, v.shape[-1]))


@jax.jit
def pallas_adaLN_cond__sliding_block_cached__mixer_gmlp__decode_kernel(
    A_x: jax.Array,
    A_k_cache: jax.Array,
    A_v_cache: jax.Array,
    A_wq: jax.Array,
    A_wo: jax.Array,
    B_x: jax.Array,
    B_w_in: jax.Array,
    B_w_sp: jax.Array,
    B_b_sp: jax.Array,
    B_w_out: jax.Array,
    c: jax.Array,
    w_mod: jax.Array,
):
    del B_x
    D = A_x.shape[-1]
    HKV, SK = A_k_cache.shape[1], A_k_cache.shape[2]
    W = min(4096, max(256, SK // 4))
    QD = _HQ * _DH
    F = B_w_in.shape[-1]
    FH = F // 2
    assert A_x.shape == (1, 1, 448) and _HQ == 2 * HKV and F == 1792 and W == 4096
    bf16, f32 = jnp.bfloat16, jnp.float32

    n_full, rem = divmod(W, _KV_ROWS)
    n_kv = n_full + (1 if rem else 0)
    wo_a_rows = 192
    win_a_rows = 224
    out_chunks = ((0, 256), (256, 128), (384, D - 384))

    def kernel(x_hbm, k_hbm, v_hbm, wq_hbm, woT_hbm, win_hbm, wsp_hbm, bsp_hbm,
               woutT_hbm, c_hbm, wmod_hbm,
               out_ref,
               x_v, c_v, wsp_v, bsp_v, wmod_v, wq_v, k_v, v_v, woT_v, win_v,
               woutT_v, q_s, o_s, mod_s):

        def body(sem_w, sem_k, sem_v, sem_out, sem_small):
            def pieces(src, dst, sem, r_lo, r_hi, r_step, c_step):
                return [(src.at[pl.ds(r, r_step), pl.ds(c0, c_step)],
                         dst.at[pl.ds(r, r_step), pl.ds(c0, c_step)], sem)
                        for r in range(r_lo, r_hi, r_step)
                        for c0 in range(0, src.shape[1], c_step)]

            def kv_piece(src, dst, sem, g, r, n):
                return (src.at[0, g, pl.ds(SK - W + r, n), :],
                        dst.at[g, pl.ds(r, n), :], sem.at[g])

            def kv_pieces(src, dst, sem, g):
                out = [kv_piece(src, dst, sem, g, j * _KV_ROWS, _KV_ROWS)
                       for j in range(n_full)]
                if rem:
                    out.append(kv_piece(src, dst, sem, g, W - rem, rem))
                return out

            def start(piece, priority):
                pltpu.make_async_copy(*piece).start(priority=priority)

            def start_pairs(a, b):
                for i in range(max(len(a), len(b))):
                    if i < len(a):
                        start(a[i], 0)
                    if i < len(b):
                        start(b[i], 1)

            def start_kv_pairs(gk, gv):
                def pair(j, carry):
                    r = pl.multiple_of(j * _KV_ROWS, 8)
                    start(kv_piece(k_hbm, k_v, sem_k, gk, r, _KV_ROWS), 0)
                    start(kv_piece(v_hbm, v_v, sem_v, gv, r, _KV_ROWS), 1)
                    return carry

                lax.fori_loop(0, n_full, pair, 0)
                if rem:
                    start(kv_piece(k_hbm, k_v, sem_k, gk, W - rem, rem), 0)
                    start(kv_piece(v_hbm, v_v, sem_v, gv, W - rem, rem), 1)

            def wait_filled(dst, sem):
                pltpu.make_async_copy(dst, dst, sem).wait()

            wmod_p = pieces(wmod_hbm, wmod_v, sem_w.at[0], 0, D, 8, 6 * D)
            wq_p = (pieces(wq_hbm, wq_v, sem_w.at[1], 0, 16, 8, 256)
                    + pieces(wq_hbm, wq_v, sem_w.at[1], 16, D, 8, QD // 2))
            wo_a = pieces(woT_hbm, woT_v, sem_w.at[2], 0, wo_a_rows, 8, QD // 2)
            wo_b = pieces(woT_hbm, woT_v, sem_w.at[2], wo_a_rows, D, 8, QD // 2)
            win_a = pieces(win_hbm, win_v, sem_w.at[3], 0, win_a_rows, 8, F)
            win_b = pieces(win_hbm, win_v, sem_w.at[3], win_a_rows, D, 8, F)
            wout_p = []
            for i, (r0, n) in enumerate(out_chunks):
                wout_p += pieces(woutT_hbm, woutT_v, sem_out.at[i], r0, r0 + n, 16, FH)
            late_a = wo_a + win_a
            late_b = wo_b + win_b + wout_p
            small = [
                pltpu.make_async_copy(c_hbm, c_v, sem_small.at[0]),
                pltpu.make_async_copy(x_hbm.at[0], x_v, sem_small.at[1]),
                pltpu.make_async_copy(wsp_hbm, wsp_v, sem_small.at[2]),
                pltpu.make_async_copy(bsp_hbm, bsp_v, sem_small.at[3]),
            ]

            nb = (len(wq_p) - len(wmod_p) - (n_kv - 1)) // 2
            first_a = wq_p[:len(wq_p) - nb]
            first_b = wmod_p + wq_p[len(wq_p) - nb:]
            start_pairs(first_a[:len(first_b)], first_b)
            start_pairs(first_a[len(first_b):], kv_pieces(v_hbm, v_v, sem_v, 0))
            for cp in small:
                cp.start()
            start_pairs(kv_pieces(k_hbm, k_v, sem_k, 0),
                        kv_pieces(v_hbm, v_v, sem_v, 1))

            for cp in small:
                cp.wait()
            wait_filled(wmod_v, sem_w.at[0])
            wait_filled(wq_v, sem_w.at[1])
            cf = c_v[...].astype(f32)
            sc = _rows(cf * jax.nn.sigmoid(cf)).astype(bf16)
            mod = jnp.dot(sc, wmod_v[...], preferred_element_type=f32)
            for i in range(6):
                mod_s[i] = mod[:, i * D:(i + 1) * D]

            x0 = _rows(x_v[...].astype(f32))
            h = (_layernorm(x0) * (1.0 + mod_s[1]) + mod_s[0]).astype(bf16)
            q = jnp.dot(h, wq_v[...], preferred_element_type=f32)
            even = (lax.broadcasted_iota(jnp.int32, (_M, _DH), 0) % 2) == 0
            for g in range(HKV):
                qa = q[:, (2 * g) * _DH:(2 * g + 1) * _DH]
                qb = q[:, (2 * g + 1) * _DH:(2 * g + 2) * _DH]
                q_s[g] = jnp.where(even, qa, qb).astype(bf16)

            n_a1 = len(wo_a)

            def head(g, carry):
                @pl.when(g + 2 < HKV)
                def _():
                    start_kv_pairs(g + 1, g + 2)

                @pl.when(g + 2 == HKV)
                def _():
                    start_pairs(kv_pieces(k_hbm, k_v, sem_k, HKV - 1), late_b[:n_kv])

                @pl.when(g + 1 == HKV)
                def _():
                    start_pairs(late_a[:n_a1], late_b[n_kv:n_kv + n_a1])

                wait_filled(k_v.at[g], sem_k.at[g])
                wait_filled(v_v.at[g], sem_v.at[g])
                s = lax.dot_general(q_s[g], k_v[g], _NT,
                                    preferred_element_type=f32) * (_DH ** -0.5)
                m = jnp.max(s, axis=-1, keepdims=True)
                p = jnp.exp(s - m)
                l = jnp.sum(p, axis=-1, keepdims=True)
                o = jnp.dot(p.astype(bf16), v_v[g], preferred_element_type=f32)
                o_s[g] = o / l
                return carry

            lax.fori_loop(0, HKV, head, 0)
            start_pairs(late_a[n_a1:], late_b[n_kv + n_a1:])

            parts = []
            for g in range(HKV):
                o = o_s[g]
                parts.append(jnp.where(even, o, 0.0))
                parts.append(jnp.where(even, 0.0, o))
            o_all = jnp.concatenate(parts, axis=-1).astype(bf16)
            wait_filled(woT_v, sem_w.at[2])
            y = lax.dot_general(o_all, woT_v[...], _NT, preferred_element_type=f32)
            y = _rows(y[0:1] + y[1:2])
            x1 = x0 + mod_s[2] * y

            h2 = (_layernorm(x1) * (1.0 + mod_s[4]) + mod_s[3]).astype(bf16)
            wait_filled(win_v, sem_w.at[3])
            z2 = _layernorm(_gelu_tanh(
                jnp.dot(h2, win_v[:, FH:], preferred_element_type=f32)))
            gate = wsp_v[...].astype(f32) * z2 + bsp_v[...].astype(f32)
            z1 = _gelu_tanh(jnp.dot(h2, win_v[:, :FH], preferred_element_type=f32))
            zg = (z1 * gate).astype(bf16)
            y2 = []
            for i, (r0, n) in enumerate(out_chunks):
                wait_filled(woutT_v.at[pl.ds(r0, n), :], sem_out.at[i])
                y2.append(lax.dot_general(zg, woutT_v[r0:r0 + n, :], _NT,
                                          preferred_element_type=f32))
            x2 = x1 + mod_s[5] * jnp.concatenate(y2, axis=-1)
            out_ref[0] = x2[0:1].astype(out_ref.dtype)

        pl.run_scoped(
            body,
            pltpu.SemaphoreType.DMA((4,)),
            pltpu.SemaphoreType.DMA((HKV,)),
            pltpu.SemaphoreType.DMA((HKV,)),
            pltpu.SemaphoreType.DMA((len(out_chunks),)),
            pltpu.SemaphoreType.DMA((4,)),
        )

    any_spec = pl.BlockSpec(memory_space=pl.ANY)
    return pl.pallas_call(
        kernel,
        out_shape=jax.ShapeDtypeStruct(A_x.shape, A_x.dtype),
        in_specs=[any_spec] * 11,
        out_specs=pl.BlockSpec(memory_space=pltpu.VMEM),
        scratch_shapes=[
            pltpu.VMEM((1, D), bf16),
            pltpu.VMEM((1, D), bf16),
            pltpu.VMEM((1, 1), bf16),
            pltpu.VMEM((1, 1), bf16),
            pltpu.VMEM((D, 6 * D), bf16),
            pltpu.VMEM((D, QD), bf16),
            pltpu.VMEM((HKV, W, _DH), bf16),
            pltpu.VMEM((HKV, W, _DH), bf16),
            pltpu.VMEM((D, QD), bf16),
            pltpu.VMEM((D, F), bf16),
            pltpu.VMEM((D, FH), bf16),
            pltpu.VMEM((HKV, _M, _DH), bf16),
            pltpu.VMEM((HKV, _M, _DH), f32),
            pltpu.VMEM((6, _M, D), f32),
        ],
        compiler_params=pltpu.CompilerParams(
            vmem_limit_bytes=100 * 1024 * 1024),
    )(A_x, A_k_cache, A_v_cache, A_wq, A_wo.T, B_w_in, B_w_sp,
      B_b_sp.reshape(1, 1), B_w_out.T, c, w_mod)
```
